```python
import os as _os
_os.environ.setdefault("JAX_PLATFORMS", "cpu")
import jax
import jax.numpy as jnp

def _softmax(x, axis=-1):
    return jax.nn.softmax(x, axis=axis)
def _gelu(x):
    return jax.nn.gelu(x, approximate=True)
def _silu(x):
    return jax.nn.silu(x)
def _sigmoid(x):
    return jax.nn.sigmoid(x)
def _layernorm(x, axis=-1, eps=1e-5):
    m = jnp.mean(x, axis=axis, keepdims=True)
    v = jnp.var(x, axis=axis, keepdims=True)
    return (x - m) / jnp.sqrt(v + eps)
def _scatter_add(tgt, idx, src, axis=0):
    return tgt.at[idx].add(src)
def _segment_sum(src, seg, n):
    return jax.ops.segment_sum(src, seg, n)
class _Rng:
    def __init__(self, key):
        self._k = key
    def _next(self):
        self._k, sub = jax.random.split(self._k)
        return sub
    def normal(self, shape):
        return jax.random.normal(self._next(), shape, dtype=jnp.bfloat16)
    def randint(self, lo, hi, shape):
        return jax.random.randint(self._next(), shape, lo, hi, dtype=jnp.int32)
    def uniform(self, shape, lo=0.0, hi=1.0):
        return jax.random.uniform(self._next(), shape, jnp.bfloat16, lo, hi)
    def permutation(self, n):
        return jax.random.permutation(self._next(), n)


kernel_name = 'concat_heads__ssm_conv_s4__sliding_local_dilated__prompt'

def setup_inputs():
    _rng = _Rng(jax.random.key(int.from_bytes(__import__("os").urandom(4), "little")))
    _w = (lambda a: (lambda t: t.astype(jnp.bfloat16) if jnp.issubdtype(t.dtype, jnp.floating) else t)(jnp.asarray(a)))
    def _A_setup():
        B, L, D, N = 1, 2048, 640, 192
        A_re = -jnp.exp((lambda *s: _rng.normal(s) * 0.8)(D, N))
        A_im = jnp.pi * (lambda *s: _rng.normal(s) * 0.8)(D, N)
        B_re = (lambda *s: _rng.normal(s) * 0.8)(D, N)
        B_im = (lambda *s: _rng.normal(s) * 0.8)(D, N)
        C_re = (lambda *s: _rng.normal(s) * 0.8)(D, N)
        C_im = (lambda *s: _rng.normal(s) * 0.8)(D, N)
        log_dt = (lambda *s: _rng.normal(s) * 0.8)(D) * 0.5 - 4.0
        Dskip = (lambda *s: _rng.normal(s) * 0.05)(D)
        return {
            "u": _w((lambda *s: _rng.normal(s) * 0.05)(B, L, D)),
            "A_re": _w(A_re),
            "A_im": _w(A_im),
            "B_re": _w(B_re),
            "B_im": _w(B_im),
            "C_re": _w(C_re),
            "C_im": _w(C_im),
            "log_dt": _w(log_dt),
            "Dskip": _w(Dskip),
        }
    _A_in = _A_setup()

    def _B_setup():
        B, S, D = 1, 2048, 640
        return {
            "x": _w((lambda *s: _rng.normal(s) * 0.2)(B, S, D)),
            "wqkv": _w((lambda *s: _rng.normal(s) * 0.2)(D, 3 * D)),
            "wo": _w((lambda *s: _rng.normal(s) * 0.05)(D, D)),
        }
    _B_in = _B_setup()

    return {
        "A_u": _A_in["u"],
        "A_A_re": _A_in["A_re"],
        "A_A_im": _A_in["A_im"],
        "A_B_re": _A_in["B_re"],
        "A_B_im": _A_in["B_im"],
        "A_C_re": _A_in["C_re"],
        "A_C_im": _A_in["C_im"],
        "A_log_dt": _A_in["log_dt"],
        "A_Dskip": _A_in["Dskip"],
        "B_x": _B_in["x"],
        "B_wqkv": _B_in["wqkv"],
        "B_wo": _B_in["wo"],
    }

def reference(A_u, A_A_re, A_A_im, A_B_re, A_B_im, A_C_re, A_C_im, A_log_dt, A_Dskip, B_x, B_wqkv, B_wo):
    def _A_ref(u, A_re, A_im, B_re, B_im, C_re, C_im, log_dt, Dskip):
        Bsz, L, D = u.shape
        dt = jnp.exp(log_dt)[:, None]
        A = A_re + 1j * A_im
        Bc = B_re + 1j * B_im
        Cc = C_re + 1j * C_im
        logdA = dt * A
        dB = dt * Bc
        l = (lambda x, dt: x.astype(dt))(jnp.arange(L), A_re.dtype)
        P = jnp.exp(logdA[:, :, None] * l[None, None, :])
        K = jnp.einsum("dn,dnl,dn->dl", Cc, P, dB).real
        L2 = 2 * L
        Kp = jnp.pad(K, ((0, 0), (0, L)))
        up = (lambda x, *d: x.transpose(*d))(u, 0, 2, 1)
        up = jnp.pad(up, ((0, 0), (0, 0), (0, L)))
        Kf = (lambda x, axes=(-2,-1): jnp.fft.rfft2(x.astype(jnp.float32), axes=axes))(Kp[:, None, :], axes=(-2, -1))
        Uf = (lambda x, axes=(-2,-1): jnp.fft.rfft2(x.astype(jnp.float32), axes=axes))(up[:, :, None, :], axes=(-2, -1))
        Yf = Uf * Kf[None, :, :, :]
        y = (lambda x, s, axes=(-2,-1): jnp.fft.irfft2(x, s=s, axes=axes).astype(jnp.bfloat16))(Yf, (1, L2), axes=(-2, -1))[:, :, 0, :L]
        y = (lambda x, *d: x.transpose(*d))(y, 0, 2, 1) + u * Dskip[None, None, :]
        return y

    def _B_ref(x, wqkv, wo):
        B, S, D = x.shape
        H = 32; Dh = D // H
        W, dil = 8, 2
        qkv = (lambda x, *d: x.transpose(*d))((x @ wqkv).reshape(B, S, 3, H, Dh), 2, 0, 3, 1, 4)
        q, k, v = qkv[0], qkv[1], qkv[2]
        scale = Dh ** -0.5
        pos = jnp.arange(S)
        off = jnp.arange(W) * dil
        idx = pos[:, None] - off[None, :]
        mask = idx >= 0
        idx_c = jnp.where(mask, idx, 0).reshape(-1)
        kg = k[:, :, idx_c, :].reshape(B, H, S, W, Dh)
        vg = v[:, :, idx_c, :].reshape(B, H, S, W, Dh)
        logits = jnp.einsum("bhsd,bhswd->bhsw", q, kg) * scale
        logits = jnp.where(mask[None, None, :, :], logits, -1e9)
        attn = _softmax(logits, axis=-1)
        o = jnp.einsum("bhsw,bhswd->bhsd", attn, vg)
        return (lambda x, *d: x.transpose(*d))(o, 0, 2, 1, 3).reshape(B, S, D) @ wo

    a = _A_ref(A_u, A_A_re, A_A_im, A_B_re, A_B_im, A_C_re, A_C_im, A_log_dt, A_Dskip)
    b = _B_ref(B_x, B_wqkv, B_wo)
    return jnp.concatenate([a, b], axis=-1)
```

```python
import numpy as np
import jax
import jax.numpy as jnp
from jax import lax
import jax.experimental.pallas as pl
import jax.experimental.pallas.tpu as pltpu

F32 = jnp.float32
BF16 = jnp.bfloat16
I32 = jnp.int32
L, D, N = 2048, 640, 192
H, DH, W, DIL = 32, 20, 8, 2
NT = D // 128
NB = L // 128
HALO = 16
SCALE = float(np.float32(DH ** -0.5).astype(BF16))

STEPS = 8
TM1 = 96
TM2 = L // STEPS - TM1
AF = 64
P2 = 160
LAG = STEPS * TM1 - NT * AF
RC = 32
OB = 2
KG0, KG1 = 3, 4
OUT_CUTS = (STEPS * P2, L - 512, L - 256, L)
assert LAG >= TM2 and P2 <= NT * AF and STEPS * P2 <= NT * AF + (STEPS - 1) * TM2
assert KG0 + NT + KG1 * STEPS == 8 * NT

P_EXP = ((1, 5), (2, 6), (3, 7), (4, 8), (258, 516), (260, 520), (262, 772), (264, 776),
         (1032, 1544), (1288, 1800))

_SIN = (3.14159264, -5.167710084, 2.550077523, -0.5982912856, 0.0776576603)
_COS = (1.0, -4.934802137, 4.05870916, -1.335212003, 0.2349373138, -0.02439632431)


def _constants():
    def words(a):
        b = a.astype(BF16).view(np.uint16).astype(np.uint32)
        return (b[..., 0::2, :] | (b[..., 1::2, :] << 16)).view(np.int32)

    phase = (-2.0 * np.pi * (2 * np.arange(128) + 0.5) / 256.0)[:, None] * np.arange(129)[None, :]
    f = np.concatenate([np.cos(phase), np.sin(phase)], 0)
    fwd = f[:, :128]
    inv = (2.0 / 256.0) * fwd.reshape(2, 16, 8, 128).transpose(1, 0, 2, 3).reshape(256, 128).T

    loc = {}
    for j, pair in enumerate(P_EXP):
        for x, a in enumerate(pair):
            for b in range(32):
                lane = 4 * (b + x + 1) + j % 4
                if j >= 8:
                    tile, lane = 4, lane + 2 * x
                elif j >= 4:
                    tile = 2 + x
                elif b < 16:
                    tile, lane = 0, lane + 60 * x
                else:
                    tile, lane = 1, lane + 68 * (1 - x)
                loc[a + 8 * b] = (tile, lane % 128)

    lag = np.arange(L).astype(np.float32).astype(BF16).astype(np.int64)
    mats, passes = [], []
    for m in range(NB):
        tiles = {}
        for e in range(1, min(129, L - 128 * m)):
            tile, lane = loc[int(lag[128 * m + e])]
            tiles.setdefault(tile, np.zeros((256, 128)))[:, lane] += f[:, e]
        patch = None
        if len(tiles) == 2:
            lo, hi = sorted(tiles)
            src = int(np.flatnonzero(tiles[lo].any(axis=0))[0])
            dst = int(np.flatnonzero(~tiles[hi].any(axis=0))[0])
            tiles[hi][:, dst] = tiles.pop(lo)[:, src]
            patch = (lo, src, dst)
        (tile, mat), = tiles.items()
        same = [i for i, other in enumerate(mats) if np.array_equal(other, mat)]
        if not same:
            mats.append(mat)
        passes.append((tile, same[0] if same else len(mats) - 1, patch))
    return words(fwd), words(inv), words(np.stack(mats)), tuple(passes), words(np.eye(128))


_FU, _G, _FK, _PASSES, _EYE = _constants()


def _cmul(a, b):
    return a[0] * b[0] - a[1] * b[1], a[0] * b[1] + a[1] * b[0]


def _csq(a):
    t = a[0] * a[1]
    return a[0] * a[0] - a[1] * a[1], t + t


def _cexp(zr, zi):
    t = zi * np.float32(0.5 / np.pi)
    r = t - jnp.round(t)
    r2 = r * r
    sn, cs = _SIN[-1], _COS[-1]
    for coef in _SIN[-2::-1]:
        sn = sn * r2 + coef
    for coef in _COS[-2::-1]:
        cs = cs * r2 + coef
    mag = jnp.exp(0.5 * zr)
    return _csq((mag * cs, (mag * r) * sn))


def _weave(*streams):
    live = [[0.0, n, gen, float(total)] for n, (gen, total) in enumerate(streams)]
    while live:
        cur = min(live, key=lambda item: item[:2])
        cost = next(cur[2], None)
        if cost is None:
            live = [item for item in live if item is not cur]
        else:
            cur[0] += cost / cur[3]


def _take(gen, amount):
    while amount > 0:
        cost = next(gen, None)
        if cost is None:
            return
        amount -= cost
        yield cost


def _run(gen):
    for _ in gen:
        pass


def _bf(words):
    return pltpu.bitcast(words, BF16)


def _words(x):
    return pltpu.bitcast(x.astype(BF16), I32)


def _dot(a, b):
    return jnp.dot(a, b, preferred_element_type=F32)


def _dot_nt(a, b):
    return lax.dot_general(a, b, (((1,), (1,)), ((), ())), preferred_element_type=F32)


def _kernel(u_h, are_h, aim_h, bre_h, bim_h, cre_h, cim_h, ldt_h, dsk_h, x_h, wqkv_h, wo_h,
            fu_h, g_h, fk_h, eye_h, out_h,
            ldt_v, dsk_v, eye_v, par_v, u_v, x_v, wqkv_v, wo_v, fu_v, g_v, fk_v,
            wt_s, wp_s, wop_s, p_s, skip_s, kc_s, qkv_s, ux_s, kf_s, oa_s, yo_s, o_s,
            sems, wsems, osems):
    xa, xb, xc = pl.ds(0, 2 * TM1), pl.ds(2 * TM1, (STEPS - 2) * TM1), pl.ds(STEPS * TM1, STEPS * TM2)
    pairs = dict(
        ldt=(ldt_h, ldt_v), dsk=(dsk_h, dsk_v), eye=(eye_h, eye_v), u=(u_h, u_v), fu=(fu_h, fu_v),
        fk=(fk_h, fk_v), g=(g_h, g_v), xa=(x_h.at[xa], x_v.at[xa]), xb=(x_h.at[xb], x_v.at[xb]),
        xc=(x_h.at[xc], x_v.at[xc]))
    for n, src in enumerate((are_h, aim_h, bre_h, bim_h, cre_h, cim_h)):
        pairs["p%d" % n] = (src, par_v.at[n])
    cps = {name: pltpu.make_async_copy(a, b, sems.at[n]) for n, (name, (a, b)) in enumerate(pairs.items())}

    def start(*names):
        for name in names:
            cps[name].start()

    def wait(*names):
        for name in names:
            cps[name].wait()

    def tile(i):
        return pl.ds(128 * i if isinstance(i, int) else pl.multiple_of(128 * i, 128), 128)

    def w_copies(i):
        return (pltpu.make_async_copy(wqkv_h.at[tile(i), :], wqkv_v.at[tile(i), :], wsems.at[i]),
                pltpu.make_async_copy(wo_h.at[:, tile(i)], wo_v.at[:, tile(i)], wsems.at[NT + i]))

    def w_start(i):
        for cp in w_copies(i):
            cp.start()

    def w_wait(i):
        for cp in w_copies(i):
            cp.wait()

    def a_copy(t0, rows):
        return pltpu.make_async_copy(
            oa_s.at[pl.ds(t0, rows), :], out_h.at[pl.ds(t0, rows), pl.ds(0, D)], osems.at[0])

    def b_copy(t0, rows):
        return pltpu.make_async_copy(
            yo_s.at[pl.ds(t0, rows), :], out_h.at[pl.ds(t0, rows), pl.ds(D, D)], osems.at[1])

    def early(p, j, t, n):
        return qkv_s.at[p * NT + j, pl.ds(HALO + t, n), :]

    def late(p, j, t, n):
        return ux_s.at[p * NT + j, pl.ds(t, n), :]

    def spec(plane, m, c):
        return pl.ds(pl.multiple_of(8 * ((3 * c + plane) * NB + m), 8), 8)

    sub = lax.broadcasted_iota(I32, (8, 128), 0)
    lan = lax.broadcasted_iota(I32, (8, 128), 1)
    low = sub < 4
    even = (sub & 1) == 0
    slot = lan & 3

    def put(i, c, val):
        p_s[pl.ds(960 * i + 128 * c, 128), :] = val[:128].T
        rest = val[128:]
        p_s[pl.ds(960 * i + D + 64 * c, 64), :] = jnp.concatenate(
            [rest, pltpu.roll(rest, 64, 1)], axis=0).T[:64]

    def mix(a, b):
        ra = [pltpu.roll(t, 4, 0) for t in a]
        rb = ra if b is a else [pltpu.roll(t, 4, 0) for t in b]
        return (tuple(jnp.where(low, a[i], rb[i]) for i in range(2)),
                tuple(jnp.where(low, ra[i], b[i]) for i in range(2)))

    def rev(t):
        return jnp.where(even, pltpu.roll(t, 1, 0), pltpu.roll(t, 3, 0))

    def factors(r):
        v = [p_s[pl.ds(pl.multiple_of(960 * k + r, 8), 8), :] for k in range(4)]
        mu, w = (v[0], v[1]), (v[2], v[3])
        m = {1: mu}
        for k in range(9):
            m[2 << k] = _csq(m[1 << k])
        w1 = _cmul(w, mu)
        w5 = _cmul(w1, m[4])
        w258 = _cmul(_cmul(w1, mu), m[256])
        w8 = _cmul(w, m[8])
        w516 = _cmul(_cmul(w, m[4]), m[512])
        w1032 = _cmul(_cmul(w8, m[512]), m[512])
        w1544 = _cmul(w1032, m[512])
        s0, s4, s8 = mix(w1, w5), mix(w258, w516), mix(w1032, w1544)
        d1, d24, d4x, d256 = mix(mu, mu), mix(m[2], m[4]), mix(m[4], m[256]), mix(m[256], m[256])
        d8, d16 = mix(m[8], m[8]), mix(m[16], m[16])
        res = []
        for h in range(2):
            p = [s0[h]]
            for _ in range(3):
                p.append(_cmul(p[-1], d1[h]))
            p.append(s4[h])
            p.append(_cmul(p[4], d24[h]))
            p.append(_cmul(p[4], d4x[h]))
            p.append(_cmul(p[5], d4x[h]))
            p.append(s8[h])
            p.append(_cmul(p[8], d256[h]))
            q = [(jnp.where(low, 1.0, rev(d8[h][0])), jnp.where(low, 0.0, -rev(d8[h][1])))]
            qm = (rev(d16[h][0]), -rev(d16[h][1]))
            for _ in range(15):
                q.append(_cmul(q[-1], qm))
            res.append((p, q))
        return res

    def mat(vals):
        return jnp.concatenate([jnp.concatenate(t, axis=1) for t in vals], axis=0).astype(BF16)

    def diag(o):
        r = [pltpu.roll(o[8 * j:8 * j + 8], j % 4 + 1, 1, stride=1, stride_axis=0) for j in range(10)]

        def merge(a):
            return jnp.where(slot == 0, a[0], jnp.where(slot == 1, a[1], jnp.where(slot == 2, a[2], a[3])))

        return merge(r[0:4]), merge(r[4:8]), jnp.where(slot == 0, r[8], r[9])

    def taps(first, count):
        for n in range(count):
            i = first + n
            fac = factors(D + 8 * i)
            yield 1
            shared = []
            for p, q in fac:
                lhs = ([[jnp.where(lan < 64, t, 0.0) for t in z] for z in p]
                       + [[jnp.where(lan < 64, 0.0, t) for t in z] for z in p])
                o = _dot_nt(mat(lhs), mat(q))
                shared.append((o[:80], o[80:]))
            for half in range(2):
                r0 = pl.multiple_of(128 * (i // 8) + 8 * (i % 8) + 64 * half, 8)
                fac = factors(r0)
                yield 1
                ms = [diag(_dot_nt(mat(p), mat(q)) + shared[h][half]) for h, (p, q) in enumerate(fac)]
                tl = []
                for a, b in zip(*ms):
                    tl.append(jnp.where(low, a, pltpu.roll(b, 4, 0)))
                    tl.append(jnp.where(low, pltpu.roll(a, 4, 0), b))
                for t in range(4):
                    kc_s[t, pl.ds(r0, 8), :] = tl[t]
                kc_s[4, pl.ds(r0, 8), :] = jnp.where(slot < 2, tl[4], pltpu.roll(tl[5], 2, 1))

    def toeplitz(v, c, plane, i0):
        acc, b = [None] * OB, []
        for m in reversed(range(i0 + OB)):
            a = kf_s[v, spec(plane, m, c), :]
            b.append(ux_s[3 * NT + v, spec(plane, len(b), c), :])
            cost = 0
            for o in range(OB):
                if i0 + o >= m:
                    t = a * b[i0 + o - m]
                    acc[o] = t if acc[o] is None else acc[o] + t
                    cost += 1
            yield cost
        return acc

    def convolve(v, c):
        for i0 in range(0, NB, OB):
            t1 = yield from toeplitz(v, c, 0, i0)
            t2 = yield from toeplitz(v, c, 1, i0)
            t3 = yield from toeplitz(v, c, 2, i0)
            for o in range(OB):
                yo_s[pl.ds(pl.multiple_of(L + 256 * (i0 + o) + 16 * v, 16), 16), tile(c)] = (
                    jnp.concatenate([t1[o] - t3[o], t1[o] + t2[o]], axis=0).astype(BF16))

    def reorder(c):
        wt_s[pl.ds(3 * D, D), :] = wo_v[:, tile(c)].astype(F32)
        for d in range(DH):
            wop_s[pl.ds(H * d // 2, H // 2), tile(c)] = _words(wt_s[pl.ds(3 * D + d, H, stride=DH), :])
        for p in range(3):
            for ct in range(NT * p, NT * p + NT):
                wt_s[tile(ct), :] = _dot_nt(_bf(eye_v[...]), wqkv_v[tile(c), tile(ct)])
                yield 1
            for d in range(DH):
                row = 384 * (d // 4) + 128 * p + H * (d % 4)
                wp_s[pl.ds(row // 2, H // 2), tile(c)] = _words(wt_s[pl.ds(D * p + d, H, stride=DH), :])

    def qkv(dests, t0, tm):
        x = x_v[pl.ds(t0, tm), :]
        for j in range(NT):
            for p in range(3):
                o = _dot_nt(x, _bf(wp_s[pl.ds(192 * j + 64 * p, 64), :]))
                for r in range(0, tm, 16):
                    for rows in dests:
                        rows(p, j, t0 + r, 16)[...] = o[r:r + 16]
                    yield 16

    def window(rows, p, j, t0):
        wide = [rows(p, j, t0 - 8 - DIL * w, RC + 8)[...] for w in range(W // 2)]
        return [t[8:] for t in wide] + [t[:RC] for t in wide]

    def attend(rows, first, tm, masked):
        for r in range(0, tm, RC):
            t0 = first + r
            parts = [None] * W
            for j in range(NT):
                q = rows(0, j, t0, RC)[...]
                for w, k in enumerate(window(rows, 1, j, t0)):
                    parts[w] = q * k if j == 0 else parts[w] + q * k
                yield 1
            lg = []
            for t in parts:
                t = t + pltpu.roll(t, 64, 1)
                lg.append(t + pltpu.roll(t, 32, 1))
            if masked and r == 0:
                pos = t0 + lax.broadcasted_iota(I32, (RC, 128), 0)
                lg = [jnp.where(pos >= DIL * w, lg[w], -1e9 / SCALE) for w in range(W)]
            mx = lg[0]
            for t in lg[1:]:
                mx = jnp.maximum(mx, t)
            e = [jnp.exp2((t - mx) * float(SCALE * np.log2(np.e))) for t in lg]
            den = e[0]
            for t in e[1:]:
                den = den + t
            inv = 1.0 / den
            for j in range(NT):
                acc = None
                for w, v in enumerate(window(rows, 2, j, t0)):
                    acc = e[w] * v if acc is None else acc + e[w] * v
                o_s[pl.ds(pl.multiple_of(t0, RC), RC), tile(j)] = (acc * inv).astype(BF16)
                yield 1

    def project(t0, tm):
        o = o_s[pl.ds(t0, tm), :]

        def gen():
            for j in range(NT):
                res = _dot(o, _bf(wop_s[:, tile(j)]))
                for r in range(0, tm, 16):
                    yo_s[pl.ds(pl.multiple_of(t0 + r, 16), 16), tile(j)] = res[r:r + 16].astype(BF16)
                    yield 16

        return gen()

    start("ldt", "p0", "p1", "dsk", "eye", "p2", "p3", "p4", "p5")
    wait("ldt")
    dt = jnp.exp(ldt_v[...].reshape(1, D).astype(F32)).astype(BF16).astype(F32)
    wait("p0", "p1")
    w_start(0)
    for c in range(NT):
        dtc = dt[:, 128 * c:128 * c + 128]
        mu = _cexp(dtc * par_v[0, :, tile(c)].astype(F32), dtc * par_v[1, :, tile(c)].astype(F32))
        put(0, c, mu[0])
        put(1, c, mu[1])
    wait("p2", "p3", "p4", "p5", "dsk")
    w_start(1)
    dskip = dsk_v[...].reshape(1, D).astype(F32)
    for c in range(NT):
        dtc = dt[:, 128 * c:128 * c + 128]
        w = _cmul((par_v[4, :, tile(c)].astype(F32), par_v[5, :, tile(c)].astype(F32)),
                  (dtc * par_v[2, :, tile(c)].astype(F32), dtc * par_v[3, :, tile(c)].astype(F32)))
        skip_s[:, tile(c)] = jnp.broadcast_to(
            dskip[:, 128 * c:128 * c + 128] + jnp.sum(w[0], axis=0, keepdims=True), (8, 128))
        put(2, c, w[0])
        put(3, c, w[1])
    w_start(2)

    def weights(i, _):
        w_wait(i)

        @pl.when(i < NT - 3)
        def _():
            w_start(i + 3)

        @pl.when(i == NT - 3)
        def _():
            start("xa", "xb")

        _weave((reorder(i), 3 * NT), (taps(KG0 + i, 1), 4))
        return 0

    wait("eye")
    w_wait(0)
    w_start(3)
    _weave((taps(0, KG0 + 1), 3 * KG0 + 3), (reorder(0), 3 * NT * 0.9))
    lax.fori_loop(1, NT, weights, 0)
    wait("xa")
    start("fk", "fu", "u", "g", "xc")

    def loop1(i, _):
        @pl.when(i == 2)
        def _():
            wait("xb")

        _weave((qkv((early, late), pl.multiple_of(TM1 * i, RC), TM1), 3 * NT * TM1),
               (taps(KG0 + NT + KG1 * i, KG1), 3 * KG1 + 2))
        return 0

    lax.fori_loop(0, STEPS, loop1, 0)
    for p in (1, 2):
        for j in range(NT):
            early(p, j, -HALO, HALO)[...] = jnp.broadcast_to(early(p, j, 0, 1)[...], (HALO, 128))
    wait("fk", "fu", "u", "g", "xc")

    def forward(c, _):
        _run(attend(early, pl.multiple_of(AF * c, RC), AF, True))
        kc = [kc_s[t, tile(c), :] for t in range(5)]
        lane = lax.broadcasted_iota(I32, (128, 128), 1)
        kc[:2] = [jnp.where((lane >= 4) & (lane < 68), kc[0], pltpu.roll(kc[1], 60, 1)),
                  jnp.where((lane >= 8) & (lane < 72), pltpu.roll(kc[0], 68, 1), kc[1])]
        prev = None
        for m in range(NB):
            t, idx, patch = _PASSES[m]
            kt = kc[t]
            if patch is not None:
                kt = jnp.where(lane == patch[2], pltpu.roll(kc[patch[0]], (patch[2] - patch[1]) % 128, 1), kt)
            kf = _dot_nt(_bf(fk_v[idx]), kt.astype(BF16))
            re, im = kf[:128], kf[128:]
            if prev is not None:
                re, im = re - prev[128:], im + prev[:128]
            prev = kf
            for plane, val in enumerate((re, im - re, im + re)):
                for v in range(16):
                    kf_s[v, spec(plane, m, c), :] = val[8 * v:8 * v + 8]
            uf = _dot(_bf(fu_v[...]), u_v[tile(m), tile(c)])
            for plane, val in enumerate((uf[:128] + uf[128:], uf[:128], uf[128:])):
                for v in range(16):
                    ux_s[3 * NT + v, spec(plane, m, c), :] = val[8 * v:8 * v + 8]
        return 0

    lax.fori_loop(0, NT, forward, 0)

    def loop2(i, _):
        t0 = pl.multiple_of(STEPS * TM1 + TM2 * i, RC)
        p0 = pl.multiple_of(P2 * i, RC)
        out = project(p0, P2)

        def dense():
            yield from out
            yield from qkv((late,), t0, TM2)

        def blocks():
            for c in range(NT):
                for n in range(16 // STEPS):
                    yield from convolve(16 // STEPS * i + n, c)

        work = blocks()
        _run(_take(work, 40))
        _weave((dense(), 0.9 * NT * (3 * TM2 + P2)), (work, 16 // STEPS * NT * 3 * 136 - 40))
        _run(attend(late, t0 - LAG, TM2, False))
        b_copy(p0, P2).start()
        return 0

    lax.fori_loop(0, STEPS, loop2, 0)

    skip = skip_s[0:1, :]

    def inverse():
        for m in range(NB):
            y = _dot(_bf(g_v[...]), yo_s[pl.ds(L + 256 * m, 256), :])
            oa_s[tile(m), :] = (y + u_v[tile(m), :].astype(F32) * skip).astype(BF16)
            a_copy(128 * m, 128).start()
            yield 1

    _weave((inverse(), NB), (attend(late, L - LAG, LAG, False), 12 * LAG / RC))
    for a, b in zip(OUT_CUTS, OUT_CUTS[1:]):
        _run(project(a, b - a))
        b_copy(a, b - a).start()
    a_copy(0, L).wait()
    b_copy(0, L).wait()


@jax.jit
def pallas_concat_heads__ssm_conv_s4__sliding_local_dilated__prompt_kernel(
    A_u: jax.Array,
    A_A_re: jax.Array,
    A_A_im: jax.Array,
    A_B_re: jax.Array,
    A_B_im: jax.Array,
    A_C_re: jax.Array,
    A_C_im: jax.Array,
    A_log_dt: jax.Array,
    A_Dskip: jax.Array,
    B_x: jax.Array,
    B_wqkv: jax.Array,
    B_wo: jax.Array,
):
    assert A_A_re.dtype == BF16 and A_u.shape == (1, L, D) and A_A_re.shape == (D, N)
    hbm = pl.BlockSpec(memory_space=pl.ANY)
    vmem = pltpu.VMEM
    out = pl.pallas_call(
        _kernel,
        out_shape=jax.ShapeDtypeStruct((L, 2 * D), BF16),
        in_specs=[hbm] * 16,
        out_specs=hbm,
        scratch_shapes=[
            vmem((D,), BF16), vmem((D,), BF16), vmem(_EYE.shape, I32), vmem((6, N, D), BF16),
            vmem((L, D), BF16), vmem((L, D), BF16), vmem((D, 3 * D), BF16), vmem((D, D), BF16),
            vmem(_FU.shape, I32), vmem(_G.shape, I32), vmem(_FK.shape, I32),
            vmem((4 * D, 128), F32), vmem((3 * D // 2, D), I32), vmem((D // 2, D), I32),
            vmem((6 * D, 128), F32), vmem((8, D), F32), vmem((5, D, 128), F32),
            vmem((3 * NT, HALO + STEPS * TM1, 128), F32), vmem((3 * NT + 16, L, 128), F32),
            vmem((16, 8 * 3 * NT * NB, 128), F32),
            vmem((L, D), BF16), vmem((3 * L, D), BF16), vmem((L, D), BF16),
            pltpu.SemaphoreType.DMA((16,)), pltpu.SemaphoreType.DMA((2 * NT,)),
            pltpu.SemaphoreType.DMA((2,)),
        ],
        compiler_params=pltpu.CompilerParams(
            vmem_limit_bytes=110 * 1024 * 1024,
            flags={"XLA_TPU_EVENLY_DISTRIBUTE_CRITICAL_NODES": True}),
        name="fused",
    )(A_u.reshape(L, D), A_A_re.T, A_A_im.T, A_B_re.T, A_B_im.T, A_C_re.T, A_C_im.T, A_log_dt, A_Dskip,
      B_x.reshape(L, D), B_wqkv, B_wo, _FU, _G, _FK, _EYE)
    return out.reshape(1, L, 2 * D)
```

```python
import numpy as np
import jax
import jax.numpy as jnp
from jax import lax
import jax.experimental.pallas as pl
import jax.experimental.pallas.tpu as pltpu

F32 = jnp.float32
BF16 = jnp.bfloat16
I32 = jnp.int32
L, D, N = 2048, 640, 192
H, DH, W, DIL = 32, 20, 8, 2
NT = D // 128
NB = L // 128
HALO = 16
SCALE = float(np.float32(DH ** -0.5).astype(BF16))

TM1 = 384
STEPS = 8
TM2 = 160
AF = 48
P2 = 160
LAG = 2 * TM1 - NT * AF
WP = 1.2
OB = 2
KG0, KG1 = 3, 16
OUT_CUTS = (STEPS * P2, L - 512, L - 256, L)
assert LAG >= TM2 and P2 <= NT * AF and STEPS * P2 <= NT * AF + (STEPS - 1) * TM2
assert KG0 + NT + 2 * KG1 == 8 * NT and 2 * TM1 + STEPS * TM2 == L

P_EXP = ((1, 5), (2, 6), (3, 7), (4, 8), (258, 516), (260, 520), (262, 772), (264, 776),
         (1032, 1544), (1288, 1800))

_SIN = (3.14159264, -5.167710084, 2.550077523, -0.5982912856, 0.0776576603)
_COS = (1.0, -4.934802137, 4.05870916, -1.335212003, 0.2349373138, -0.02439632431)


def _constants():
    def words(a):
        b = a.astype(BF16).view(np.uint16).astype(np.uint32)
        return (b[..., 0::2, :] | (b[..., 1::2, :] << 16)).view(np.int32)

    phase = (-2.0 * np.pi * (2 * np.arange(128) + 0.5) / 256.0)[:, None] * np.arange(129)[None, :]
    f = np.concatenate([np.cos(phase), np.sin(phase)], 0)
    fwd = f[:, :128]
    inv = (2.0 / 256.0) * fwd.reshape(2, 16, 8, 128).transpose(1, 0, 2, 3).reshape(256, 128).T

    loc = {}
    for j, pair in enumerate(P_EXP):
        for x, a in enumerate(pair):
            for b in range(32):
                lane = 4 * (b + x + 1) + j % 4
                if j >= 8:
                    tile, lane = 4, lane + 2 * x
                elif j >= 4:
                    tile = 2 + x
                elif b < 16:
                    tile, lane = 0, lane + 60 * x
                else:
                    tile, lane = 1, lane + 68 * (1 - x)
                loc[a + 8 * b] = (tile, lane % 128)

    lag = np.arange(L).astype(np.float32).astype(BF16).astype(np.int64)
    mats, passes = [], []
    for m in range(NB):
        tiles = {}
        for e in range(1, min(129, L - 128 * m)):
            tile, lane = loc[int(lag[128 * m + e])]
            tiles.setdefault(tile, np.zeros((256, 128)))[:, lane] += f[:, e]
        patch = None
        if len(tiles) == 2:
            lo, hi = sorted(tiles)
            src = int(np.flatnonzero(tiles[lo].any(axis=0))[0])
            dst = int(np.flatnonzero(~tiles[hi].any(axis=0))[0])
            tiles[hi][:, dst] = tiles.pop(lo)[:, src]
            patch = (lo, src, dst)
        (tile, mat), = tiles.items()
        same = [i for i, other in enumerate(mats) if np.array_equal(other, mat)]
        if not same:
            mats.append(mat)
        passes.append((tile, same[0] if same else len(mats) - 1, patch))
    return words(fwd), words(inv), words(np.stack(mats)), tuple(passes), words(np.eye(128))


_FU, _G, _FK, _PASSES, _EYE = _constants()


def _cmul(a, b):
    return a[0] * b[0] - a[1] * b[1], a[0] * b[1] + a[1] * b[0]


def _csq(a):
    t = a[0] * a[1]
    return a[0] * a[0] - a[1] * a[1], t + t


def _cexp(zr, zi):
    t = zi * np.float32(0.5 / np.pi)
    r = t - jnp.round(t)
    r2 = r * r
    sn, cs = _SIN[-1], _COS[-1]
    for coef in _SIN[-2::-1]:
        sn = sn * r2 + coef
    for coef in _COS[-2::-1]:
        cs = cs * r2 + coef
    mag = jnp.exp(0.5 * zr)
    return _csq((mag * cs, (mag * r) * sn))


def _weave(*streams):
    live = [[0.0, n, gen, float(total)] for n, (gen, total) in enumerate(streams)]
    while live:
        cur = min(live, key=lambda item: item[:2])
        cost = next(cur[2], None)
        if cost is None:
            live = [item for item in live if item is not cur]
        else:
            cur[0] += cost / cur[3]


def _take(gen, amount):
    while amount > 0:
        cost = next(gen, None)
        if cost is None:
            return
        amount -= cost
        yield cost


def _run(gen):
    for _ in gen:
        pass


def _bf(words):
    return pltpu.bitcast(words, BF16)


def _words(x):
    return pltpu.bitcast(x.astype(BF16), I32)


def _dot(a, b):
    return jnp.dot(a, b, preferred_element_type=F32)


def _dot_nt(a, b):
    return lax.dot_general(a, b, (((1,), (1,)), ((), ())), preferred_element_type=F32)


def _kernel(u_h, are_h, aim_h, bre_h, bim_h, cre_h, cim_h, ldt_h, dsk_h, x_h, wqkv_h, wo_h,
            fu_h, g_h, fk_h, eye_h, out_h,
            ldt_v, dsk_v, eye_v, par_v, u_v, x_v, wqkv_v, wo_v, fu_v, g_v, fk_v,
            wt_s, wp_s, wop_s, p_s, skip_s, kc_s, qkv_s, ux_s, kf_s, oa_s, yo_s, o_s,
            sems, wsems, osems):
    xa, xb, xc = pl.ds(0, TM1), pl.ds(TM1, TM1), pl.ds(2 * TM1, STEPS * TM2)
    pairs = dict(
        ldt=(ldt_h, ldt_v), dsk=(dsk_h, dsk_v), eye=(eye_h, eye_v), u=(u_h, u_v), fu=(fu_h, fu_v),
        fk=(fk_h, fk_v), g=(g_h, g_v), xa=(x_h.at[xa], x_v.at[xa]), xb=(x_h.at[xb], x_v.at[xb]),
        xc=(x_h.at[xc], x_v.at[xc]))
    for n, src in enumerate((are_h, aim_h, bre_h, bim_h, cre_h, cim_h)):
        pairs["p%d" % n] = (src, par_v.at[n])
    cps = {name: pltpu.make_async_copy(a, b, sems.at[n]) for n, (name, (a, b)) in enumerate(pairs.items())}

    def start(*names):
        for name in names:
            cps[name].start()

    def wait(*names):
        for name in names:
            cps[name].wait()

    def tile(i):
        return pl.ds(128 * i if isinstance(i, int) else pl.multiple_of(128 * i, 128), 128)

    def w_copies(i):
        return (pltpu.make_async_copy(wqkv_h.at[tile(i), :], wqkv_v.at[tile(i), :], wsems.at[i]),
                pltpu.make_async_copy(wo_h.at[:, tile(i)], wo_v.at[:, tile(i)], wsems.at[NT + i]))

    def w_start(i):
        for cp in w_copies(i):
            cp.start()

    def w_wait(i):
        for cp in w_copies(i):
            cp.wait()

    def a_copy(t0, rows):
        return pltpu.make_async_copy(
            oa_s.at[pl.ds(t0, rows), :], out_h.at[pl.ds(t0, rows), pl.ds(0, D)], osems.at[0])

    def b_copy(t0, rows):
        return pltpu.make_async_copy(
            yo_s.at[pl.ds(t0, rows), :], out_h.at[pl.ds(t0, rows), pl.ds(D, D)], osems.at[1])

    def early(p, j, t, n):
        return qkv_s.at[p * NT + j, pl.ds(HALO + t, n), :]

    def late(p, j, t, n):
        return ux_s.at[p * NT + j, pl.ds(t, n), :]

    def spec(plane, m, c):
        return pl.ds(pl.multiple_of(8 * ((3 * c + plane) * NB + m), 8), 8)

    sub = lax.broadcasted_iota(I32, (8, 128), 0)
    lan = lax.broadcasted_iota(I32, (8, 128), 1)
    low = sub < 4
    even = (sub & 1) == 0
    slot = lan & 3

    def put(i, c, val):
        p_s[pl.ds(960 * i + 128 * c, 128), :] = val[:128].T
        rest = val[128:]
        p_s[pl.ds(960 * i + D + 64 * c, 64), :] = jnp.concatenate(
            [rest, pltpu.roll(rest, 64, 1)], axis=0).T[:64]

    def mix(a, b):
        ra = [pltpu.roll(t, 4, 0) for t in a]
        rb = ra if b is a else [pltpu.roll(t, 4, 0) for t in b]
        return (tuple(jnp.where(low, a[i], rb[i]) for i in range(2)),
                tuple(jnp.where(low, ra[i], b[i]) for i in range(2)))

    def rev(t):
        return jnp.where(even, pltpu.roll(t, 1, 0), pltpu.roll(t, 3, 0))

    def factors(r):
        v = [p_s[pl.ds(pl.multiple_of(960 * k + r, 8), 8), :] for k in range(4)]
        mu, w = (v[0], v[1]), (v[2], v[3])
        m = {1: mu}
        for k in range(9):
            m[2 << k] = _csq(m[1 << k])
        w1 = _cmul(w, mu)
        w5 = _cmul(w1, m[4])
        w258 = _cmul(_cmul(w1, mu), m[256])
        w8 = _cmul(w, m[8])
        w516 = _cmul(_cmul(w, m[4]), m[512])
        w1032 = _cmul(_cmul(w8, m[512]), m[512])
        w1544 = _cmul(w1032, m[512])
        s0, s4, s8 = mix(w1, w5), mix(w258, w516), mix(w1032, w1544)
        d1, d24, d4x, d256 = mix(mu, mu), mix(m[2], m[4]), mix(m[4], m[256]), mix(m[256], m[256])
        d8, d16 = mix(m[8], m[8]), mix(m[16], m[16])
        res = []
        for h in range(2):
            p = [s0[h]]
            for _ in range(3):
                p.append(_cmul(p[-1], d1[h]))
            p.append(s4[h])
            p.append(_cmul(p[4], d24[h]))
            p.append(_cmul(p[4], d4x[h]))
            p.append(_cmul(p[5], d4x[h]))
            p.append(s8[h])
            p.append(_cmul(p[8], d256[h]))
            q = [(jnp.where(low, 1.0, rev(d8[h][0])), jnp.where(low, 0.0, -rev(d8[h][1])))]
            qm = (rev(d16[h][0]), -rev(d16[h][1]))
            for _ in range(15):
                q.append(_cmul(q[-1], qm))
            res.append((p, q))
        return res

    def mat(vals):
        return jnp.concatenate([jnp.concatenate(t, axis=1) for t in vals], axis=0).astype(BF16)

    def diag(o):
        r = [pltpu.roll(o[8 * j:8 * j + 8], j % 4 + 1, 1, stride=1, stride_axis=0) for j in range(10)]

        def merge(a):
            return jnp.where(slot == 0, a[0], jnp.where(slot == 1, a[1], jnp.where(slot == 2, a[2], a[3])))

        return merge(r[0:4]), merge(r[4:8]), jnp.where(slot == 0, r[8], r[9])

    def taps(first, count):
        for n in range(count):
            i = first + n
            fac = factors(D + 8 * i)
            yield 1
            shared = []
            for p, q in fac:
                lhs = ([[jnp.where(lan < 64, t, 0.0) for t in z] for z in p]
                       + [[jnp.where(lan < 64, 0.0, t) for t in z] for z in p])
                o = _dot_nt(mat(lhs), mat(q))
                shared.append((o[:80], o[80:]))
            for half in range(2):
                r0 = pl.multiple_of(128 * (i // 8) + 8 * (i % 8) + 64 * half, 8)
                fac = factors(r0)
                yield 1
                ms = [diag(_dot_nt(mat(p), mat(q)) + shared[h][half]) for h, (p, q) in enumerate(fac)]
                tl = []
                for a, b in zip(*ms):
                    tl.append(jnp.where(low, a, pltpu.roll(b, 4, 0)))
                    tl.append(jnp.where(low, pltpu.roll(a, 4, 0), b))
                for t in range(4):
                    kc_s[t, pl.ds(r0, 8), :] = tl[t]
                kc_s[4, pl.ds(r0, 8), :] = jnp.where(slot < 2, tl[4], pltpu.roll(tl[5], 2, 1))

    def toeplitz(v, c, plane, i0):
        acc, b = [None] * OB, []
        for m in reversed(range(i0 + OB)):
            a = kf_s[v, spec(plane, m, c), :]
            b.append(ux_s[3 * NT + v, spec(plane, len(b), c), :])
            cost = 0
            for o in range(OB):
                if i0 + o >= m:
                    t = a * b[i0 + o - m]
                    acc[o] = t if acc[o] is None else acc[o] + t
                    cost += 1
            yield cost
        return acc

    def convolve(v, c):
        for i0 in range(0, NB, OB):
            t1 = yield from toeplitz(v, c, 0, i0)
            t2 = yield from toeplitz(v, c, 1, i0)
            t3 = yield from toeplitz(v, c, 2, i0)
            for o in range(OB):
                yo_s[pl.ds(pl.multiple_of(L + 256 * (i0 + o) + 16 * v, 16), 16), tile(c)] = (
                    jnp.concatenate([t1[o] - t3[o], t1[o] + t2[o]], axis=0).astype(BF16))

    def reorder(c):
        wt_s[pl.ds(3 * D, D), :] = wo_v[:, tile(c)].astype(F32)
        for d in range(DH):
            wop_s[pl.ds(H * d // 2, H // 2), tile(c)] = _words(wt_s[pl.ds(3 * D + d, H, stride=DH), :])
        for p in range(3):
            for ct in range(NT * p, NT * p + NT):
                wt_s[tile(ct), :] = _dot_nt(_bf(eye_v[...]), wqkv_v[tile(c), tile(ct)])
                yield 1
            for d in range(DH):
                row = 384 * (d // 4) + 128 * p + H * (d % 4)
                wp_s[pl.ds(row // 2, H // 2), tile(c)] = _words(wt_s[pl.ds(D * p + d, H, stride=DH), :])

    def qkv(dests, t0, tm):
        x = x_v[pl.ds(t0, tm), :]
        for j in range(NT):
            for p in range(3):
                o = _dot_nt(x, _bf(wp_s[pl.ds(192 * j + 64 * p, 64), :]))
                for r in range(0, tm, 16):
                    for rows in dests:
                        rows(p, j, t0 + r, 16)[...] = o[r:r + 16]
                    yield 16

    def window(rows, p, j, t0, rc):
        wide = [rows(p, j, t0 - 8 - DIL * w, rc + 8)[...] for w in range(W // 2)]
        return [t[8:] for t in wide] + [t[:rc] for t in wide]

    def attend(rows, first, tm, masked, rc):
        for r in range(0, tm, rc):
            t0 = first + r
            parts = [None] * W
            for j in range(NT):
                q = rows(0, j, t0, rc)[...]
                for w, k in enumerate(window(rows, 1, j, t0, rc)):
                    parts[w] = q * k if j == 0 else parts[w] + q * k
                yield 1
            lg = []
            for t in parts:
                t = t + pltpu.roll(t, 64, 1)
                lg.append(t + pltpu.roll(t, 32, 1))
            if masked and r == 0:
                pos = t0 + lax.broadcasted_iota(I32, (rc, 128), 0)
                lg = [jnp.where(pos >= DIL * w, lg[w], -1e9 / SCALE) for w in range(W)]
            mx = lg[0]
            for t in lg[1:]:
                mx = jnp.maximum(mx, t)
            e = [jnp.exp2((t - mx) * float(SCALE * np.log2(np.e))) for t in lg]
            den = e[0]
            for t in e[1:]:
                den = den + t
            inv = 1.0 / den
            for j in range(NT):
                acc = None
                for w, v in enumerate(window(rows, 2, j, t0, rc)):
                    acc = e[w] * v if acc is None else acc + e[w] * v
                o_s[pl.ds(pl.multiple_of(t0, 16), rc), tile(j)] = (acc * inv).astype(BF16)
                yield 1

    def project(t0, tm):
        o = o_s[pl.ds(t0, tm), :]

        def gen():
            for j in range(NT):
                res = _dot(o, _bf(wop_s[:, tile(j)]))
                for r in range(0, tm, 16):
                    yo_s[pl.ds(pl.multiple_of(t0 + r, 16), 16), tile(j)] = res[r:r + 16].astype(BF16)
                    yield 16 * WP

        return gen()

    start("ldt", "p0", "p1", "dsk", "eye", "p2", "p3", "p4", "p5")
    wait("ldt")
    dt = jnp.exp(ldt_v[...].reshape(1, D).astype(F32)).astype(BF16).astype(F32)
    wait("p0", "p1")
    w_start(0)
    for c in range(NT):
        dtc = dt[:, 128 * c:128 * c + 128]
        mu = _cexp(dtc * par_v[0, :, tile(c)].astype(F32), dtc * par_v[1, :, tile(c)].astype(F32))
        put(0, c, mu[0])
        put(1, c, mu[1])
    wait("p2", "p3", "p4", "p5", "dsk")
    w_start(1)
    dskip = dsk_v[...].reshape(1, D).astype(F32)
    for c in range(NT):
        dtc = dt[:, 128 * c:128 * c + 128]
        w = _cmul((par_v[4, :, tile(c)].astype(F32), par_v[5, :, tile(c)].astype(F32)),
                  (dtc * par_v[2, :, tile(c)].astype(F32), dtc * par_v[3, :, tile(c)].astype(F32)))
        skip_s[:, tile(c)] = jnp.broadcast_to(
            dskip[:, 128 * c:128 * c + 128] + jnp.sum(w[0], axis=0, keepdims=True), (8, 128))
        put(2, c, w[0])
        put(3, c, w[1])
    w_start(2)

    def weights(i, _):
        w_wait(i)

        @pl.when(i < NT - 3)
        def _():
            w_start(i + 3)

        @pl.when(i == NT - 3)
        def _():
            start("xa", "xb")

        _weave((reorder(i), 3 * NT), (taps(KG0 + i, 1), 4))
        return 0

    wait("eye")
    w_wait(0)
    w_start(3)
    _weave((taps(0, KG0 + 1), 3 * KG0 + 3), (reorder(0), 3 * NT * 0.9))
    lax.fori_loop(1, NT, weights, 0)
    wait("xa")
    start("fk", "fu", "u", "g", "xc")

    def loop1(i, _):
        @pl.when(i == 1)
        def _():
            wait("xb")

        def dense():
            t0 = pl.multiple_of(TM1 * i, 128)
            for r in range(0, TM1, 128):
                yield from qkv((early, late), t0 + r, 128)

        _weave((dense(), 3 * NT * TM1), (taps(KG0 + NT + KG1 * i, KG1), 3 * KG1 + 2))
        return 0

    lax.fori_loop(0, 2, loop1, 0)
    for p in (1, 2):
        for j in range(NT):
            early(p, j, -HALO, HALO)[...] = jnp.broadcast_to(early(p, j, 0, 1)[...], (HALO, 128))
    wait("fk", "fu", "u", "g", "xc")

    def forward(c, _):
        _run(attend(early, pl.multiple_of(AF * c, 16), AF, True, 16))
        kc = [kc_s[t, tile(c), :] for t in range(5)]
        lane = lax.broadcasted_iota(I32, (128, 128), 1)
        kc[:2] = [jnp.where((lane >= 4) & (lane < 68), kc[0], pltpu.roll(kc[1], 60, 1)),
                  jnp.where((lane >= 8) & (lane < 72), pltpu.roll(kc[0], 68, 1), kc[1])]
        prev = None
        for m in range(NB):
            t, idx, patch = _PASSES[m]
            kt = kc[t]
            if patch is not None:
                kt = jnp.where(lane == patch[2], pltpu.roll(kc[patch[0]], (patch[2] - patch[1]) % 128, 1), kt)
            kf = _dot_nt(_bf(fk_v[idx]), kt.astype(BF16))
            re, im = kf[:128], kf[128:]
            if prev is not None:
                re, im = re - prev[128:], im + prev[:128]
            prev = kf
            for plane, val in enumerate((re, im - re, im + re)):
                for v in range(16):
                    kf_s[v, spec(plane, m, c), :] = val[8 * v:8 * v + 8]
            uf = _dot(_bf(fu_v[...]), u_v[tile(m), tile(c)])
            for plane, val in enumerate((uf[:128] + uf[128:], uf[:128], uf[128:])):
                for v in range(16):
                    ux_s[3 * NT + v, spec(plane, m, c), :] = val[8 * v:8 * v + 8]
        return 0

    lax.fori_loop(0, NT, forward, 0, unroll=NT)

    def loop2(i, _):
        t0 = pl.multiple_of(2 * TM1 + TM2 * i, 32)
        p0 = pl.multiple_of(P2 * i, 16)
        out = project(p0, P2)

        def dense():
            yield from out
            yield from qkv((late,), t0, TM2)

        def blocks():
            for c in range(NT):
                for n in range(16 // STEPS):
                    yield from convolve(16 // STEPS * i + n, c)

        work = blocks()
        _run(_take(work, 40))
        _weave((dense(), 0.9 * NT * (3 * TM2 + P2 * WP)), (work, 16 // STEPS * NT * 3 * 136 - 40))
        _run(attend(late, t0 - LAG, TM2, False, 32))
        b_copy(p0, P2).start()
        return 0

    lax.fori_loop(0, STEPS, loop2, 0)

    skip = skip_s[0:1, :]

    def inverse():
        for m in range(NB):
            y = _dot(_bf(g_v[...]), yo_s[pl.ds(L + 256 * m, 256), :])
            oa_s[tile(m), :] = (y + u_v[tile(m), :].astype(F32) * skip).astype(BF16)
            a_copy(128 * m, 128).start()
            yield 1

    _weave((inverse(), NB), (attend(late, L - LAG, LAG, False, 16), 12 * LAG / 16))
    for a, b in zip(OUT_CUTS, OUT_CUTS[1:]):
        _run(project(a, b - a))
        b_copy(a, b - a).start()
    a_copy(0, L).wait()
    b_copy(0, L).wait()


@jax.jit
def pallas_concat_heads__ssm_conv_s4__sliding_local_dilated__prompt_kernel(
    A_u: jax.Array,
    A_A_re: jax.Array,
    A_A_im: jax.Array,
    A_B_re: jax.Array,
    A_B_im: jax.Array,
    A_C_re: jax.Array,
    A_C_im: jax.Array,
    A_log_dt: jax.Array,
    A_Dskip: jax.Array,
    B_x: jax.Array,
    B_wqkv: jax.Array,
    B_wo: jax.Array,
):
    assert A_A_re.dtype == BF16 and A_u.shape == (1, L, D) and A_A_re.shape == (D, N)
    hbm = pl.BlockSpec(memory_space=pl.ANY)
    vmem = pltpu.VMEM
    out = pl.pallas_call(
        _kernel,
        out_shape=jax.ShapeDtypeStruct((L, 2 * D), BF16),
        in_specs=[hbm] * 16,
        out_specs=hbm,
        scratch_shapes=[
            vmem((D,), BF16), vmem((D,), BF16), vmem(_EYE.shape, I32), vmem((6, N, D), BF16),
            vmem((L, D), BF16), vmem((L, D), BF16), vmem((D, 3 * D), BF16), vmem((D, D), BF16),
            vmem(_FU.shape, I32), vmem(_G.shape, I32), vmem(_FK.shape, I32),
            vmem((4 * D + H, 128), F32), vmem((3 * D // 2, D), I32), vmem((D // 2, D), I32),
            vmem((6 * D, 128), F32), vmem((8, D), F32), vmem((5, D, 128), F32),
            vmem((3 * NT, HALO + 2 * TM1, 128), F32), vmem((3 * NT + 16, L, 128), F32),
            vmem((16, 8 * 3 * NT * NB, 128), F32),
            vmem((L, D), BF16), vmem((3 * L, D), BF16), vmem((L, D), BF16),
            pltpu.SemaphoreType.DMA((16,)), pltpu.SemaphoreType.DMA((2 * NT,)),
            pltpu.SemaphoreType.DMA((2,)),
        ],
        compiler_params=pltpu.CompilerParams(
            vmem_limit_bytes=110 * 1024 * 1024,
            flags={"XLA_TPU_EVENLY_DISTRIBUTE_CRITICAL_NODES": True}),
        name="fused",
    )(A_u.reshape(L, D), A_A_re.T, A_A_im.T, A_B_re.T, A_B_im.T, A_C_re.T, A_C_im.T, A_log_dt, A_Dskip,
      B_x.reshape(L, D), B_wqkv, B_wo, _FU, _G, _FK, _EYE)
    return out.reshape(1, L, 2 * D)
```
